```python
import os as _os
_os.environ.setdefault('JAX_PLATFORMS', 'cpu')
import jax
import jax.numpy as jnp

def _softmax(x, axis=-1):
    return jax.nn.softmax(x, axis=axis)

def _gelu(x):
    return jax.nn.gelu(x, approximate=True)

def _silu(x):
    return jax.nn.silu(x)

def _sigmoid(x):
    return jax.nn.sigmoid(x)

def _layernorm(x, axis=-1, eps=1e-05):
    m = jnp.mean(x, axis=axis, keepdims=True)
    v = jnp.var(x, axis=axis, keepdims=True)
    return (x - m) / jnp.sqrt(v + eps)

def _scatter_add(tgt, idx, src, axis=0):
    return tgt.at[idx].add(src)

def _segment_sum(src, seg, n):
    return jax.ops.segment_sum(src, seg, n)

class _Rng:

    def __init__(self, key):
        self._k = key

    def _next(self):
        self._k, sub = jax.random.split(self._k)
        return sub

    def normal(self, shape):
        return jax.random.normal(self._next(), shape, dtype=jnp.bfloat16)

    def randint(self, lo, hi, shape):
        return jax.random.randint(self._next(), shape, lo, hi, dtype=jnp.int32)

    def uniform(self, shape, lo=0.0, hi=1.0):
        return jax.random.uniform(self._next(), shape, jnp.bfloat16, lo, hi)

    def permutation(self, n):
        return jax.random.permutation(self._next(), n)
kernel_name = 'adaLN_cond__linear_kernel_hedgehog__geglu_ffn__prompt'

def setup_inputs():
    _rng = _Rng(jax.random.key(int.from_bytes(__import__("os").urandom(4), "little")))
    _w = lambda a: (lambda t: t.astype(jnp.bfloat16) if jnp.issubdtype(t.dtype, jnp.floating) else t)(jnp.asarray(a))

    def _A_setup():
        B, S, D, H = (1, 2048, 512, 32)
        Dh = D // H
        return {'x': _w((lambda *s: _rng.normal(s) * 0.05)(B, S, D)), 'wqkv': _w((lambda *s: _rng.normal(s) * 0.4)(D, 3 * D)), 'w_phi': _w((lambda *s: _rng.normal(s) * 0.4)(H, Dh, Dh) * Dh ** (-0.5)), 'wo': _w((lambda *s: _rng.normal(s) * 0.05)(D, D))}
    _A_in = _A_setup()

    def _B_setup():
        B, S, D, F = (1, 2048, 512, 1792)
        return {'x': _w((lambda *s: _rng.normal(s) * 0.05)(B, S, D)), 'w_gate': _w((lambda *s: _rng.normal(s) * 0.05)(D, F)), 'w_up': _w((lambda *s: _rng.normal(s) * 0.05)(D, F)), 'w_down': _w((lambda *s: _rng.normal(s) * 0.05)(F, D))}
    _B_in = _B_setup()
    return {'A_x': _A_in['x'], 'A_wqkv': _A_in['wqkv'], 'A_w_phi': _A_in['w_phi'], 'A_wo': _A_in['wo'], 'B_x': _B_in['x'], 'B_w_gate': _B_in['w_gate'], 'B_w_up': _B_in['w_up'], 'B_w_down': _B_in['w_down'], 'c': _w((lambda *s: _rng.normal(s) * 0.05)(1, 512) * 8.0), 'w_mod': _w((lambda *s: _rng.normal(s) * 0.05)(512, 6 * 512) * 512 ** (-0.5) * 8.0)}

def reference(A_x, A_wqkv, A_w_phi, A_wo, B_x, B_w_gate, B_w_up, B_w_down, c, w_mod):

    def _A_ref(x, wqkv, w_phi, wo):
        B, S, D = x.shape
        H = 32
        Dh = D // H
        qkv = (lambda x, *d: x.transpose(*d))((x @ wqkv).reshape(B, S, 3, H, Dh), 2, 0, 3, 1, 4)
        q, k, v = (qkv[0], qkv[1], qkv[2])
        pq = jnp.einsum('bhsd,hdf->bhsf', q, w_phi)
        pk = jnp.einsum('bhsd,hdf->bhsf', k, w_phi)
        phi_q = jnp.concatenate([_softmax(pq, axis=-1), _softmax(-pq, axis=-1)], axis=-1)
        phi_k = jnp.concatenate([_softmax(pk, axis=-1), _softmax(-pk, axis=-1)], axis=-1)
        kv = jnp.einsum('bhsf,bhsd->bhfd', phi_k, v)
        z = jnp.einsum('bhsf->bhf', phi_k)
        num = jnp.einsum('bhqf,bhfd->bhqd', phi_q, kv)
        den = jnp.einsum('bhqf,bhf->bhq', phi_q, z)[..., None] + 1e-06
        o = num / den
        return (lambda x, *d: x.transpose(*d))(o, 0, 2, 1, 3).reshape(B, S, D) @ wo

    def _B_ref(x, w_gate, w_up, w_down):
        return _gelu(x @ w_gate) * (x @ w_up) @ w_down
    x = A_x
    mod = (_silu(c) @ w_mod).reshape(c.shape[0], 6, 1, -1)
    sa, ca, ga, sb, cb, gb = (mod[:, 0].copy(), mod[:, 1].copy(), mod[:, 2].copy(), mod[:, 3].copy(), mod[:, 4].copy(), mod[:, 5].copy())
    h = _layernorm(x, axis=-1) * (1 + ca) + sa
    x = x + ga * _A_ref(h, A_wqkv, A_w_phi, A_wo)
    h = _layernorm(x, axis=-1) * (1 + cb) + sb
    x = x + gb * _B_ref(h, B_w_gate, B_w_up, B_w_down)
    return x
```

```python
import jax
import jax.numpy as jnp
from jax import lax
import jax.experimental.pallas as pl
import jax.experimental.pallas.tpu as pltpu

S, D, H, DH, F = 2048, 512, 32, 16, 1792
T = 1024
N = S // T
FC = 256
U = 256
U2 = 256
G = 4
f32, bf16 = jnp.float32, jnp.bfloat16
NT = (((1,), (1,)), ((), ()))
TN = (((0,), (0,)), ((), ()))


def _ln(x):
    m = jnp.mean(x, axis=-1, keepdims=True)
    xc = x - m
    v = jnp.mean(xc * xc, axis=-1, keepdims=True)
    return xc * lax.rsqrt(v + 1e-5)


def _phi(p):
    s = [p[8 * f:8 * f + 8] for f in range(8)]
    mx, mn = s[0], s[0]
    for a in s[1:]:
        mx = jnp.maximum(mx, a)
        mn = jnp.minimum(mn, a)
    mx = jnp.maximum(mx, pltpu.roll(mx, 4, 0))
    mn = jnp.minimum(mn, pltpu.roll(mn, 4, 0))
    out = []
    for e in ([jnp.exp2(a - mx) for a in s], [jnp.exp2(mn - a) for a in s]):
        t = e[0]
        for a in e[1:]:
            t = t + a
        r = 1.0 / (t + pltpu.roll(t, 4, 0))
        out += [a * r for a in e]
    return out


def _kernel(x_ref, c_ref, wphi_ref, wqkv_h, wmod_h, wo_h, wg_h, wu_h, wd_h, o_h,
            wqkv, wmod, wo, wg, wu, wd, wt, mod, kv, kvt, z, pk, pq, ot, o_ref_x, hb, act, tm, hs, os_, sem, osem):
    i = pl.program_id(0)

    def cps():
        return [
            pltpu.make_async_copy(wmod_h.at[:, :2 * D], wmod.at[:, :2 * D], sem.at[0]),
            pltpu.make_async_copy(wqkv_h.at[:, D:], wqkv.at[:, D:], sem.at[1]),
            pltpu.make_async_copy(wqkv_h.at[:, :D], wqkv.at[:, :D], sem.at[7]),
            pltpu.make_async_copy(wmod_h.at[:, 2 * D:], wmod.at[:, 2 * D:], sem.at[2]),
            pltpu.make_async_copy(wo_h, wo, sem.at[3]),
            pltpu.make_async_copy(wg_h, wg, sem.at[4]),
            pltpu.make_async_copy(wu_h, wu, sem.at[5]),
            pltpu.make_async_copy(wd_h, wd, sem.at[6]),
        ]

    def ocp(j, p):
        lo, n = (0, T - U2) if p == 0 else (T - U2, U2)
        return pltpu.make_async_copy(os_.at[j, pl.ds(lo, n)],
                                     o_h.at[0, pl.ds(j * T + lo, n)], osem.at[p, j])

    def silu_c():
        c = jnp.broadcast_to(c_ref[...].astype(f32), (8, D))
        return (c * jax.nn.sigmoid(c)).astype(bf16)

    r = lax.broadcasted_iota(jnp.int32, (128, 128), 0)
    l = lax.broadcasted_iota(jnp.int32, (128, 128), 1)

    hm = ((r >> 6) * 4 + (r & 3)) == (l >> 4)

    def perm():
        return ((((r >> 2) & 15) == (l & 15)) & hm).astype(bf16)

    def fold(j):
        for g in range(G):
            o = j * D + 128 * g
            wt[o:o + 128, :] = ((1.4426950408889634 if j < 2 else 1.0) * lax.dot_general(
                tm[g] if j < 2 else perm(), wqkv[:, o:o + 128], NT,
                preferred_element_type=f32)).astype(bf16)

    @pl.when(i == 0)
    def _():
        cp = cps()
        cp[1].start()
        kv[...] = jnp.zeros_like(kv)
        e = (((lax.broadcasted_iota(jnp.int32, (128, DH), 0) >> 2) & 15)
             == lax.broadcasted_iota(jnp.int32, (128, DH), 1)).astype(bf16)
        cp[0].start()
        wp = wphi_ref[...].reshape(DH * DH, H)
        for g in range(G):
            sel = (lax.broadcasted_iota(jnp.int32, (H, 128), 0) - 8 * g
                   == (lax.broadcasted_iota(jnp.int32, (H, 128), 1) >> 4)).astype(bf16)
            xx = jnp.dot(wp, sel, preferred_element_type=f32)
            dl = lax.broadcasted_iota(jnp.int32, (DH, 128), 1) & 15
            w = xx[:DH]
            for d in range(1, DH):
                w = jnp.where(dl == d, xx[DH * d:DH * d + DH], w)
            t = jnp.dot(e, w.astype(bf16), preferred_element_type=f32)
            tm[g] = jnp.where(hm, t, 0.0).astype(bf16)
        cp[1].wait()
        fold(1)
        fold(2)
        cp[0].wait()
        for a in cp[2:]:
            a.start()
        mod[:, :2 * D] = jnp.dot(silu_c(), wmod[:, :2 * D], preferred_element_type=f32)

    def hid():
        return (_ln(x_ref[...].astype(f32)) * (1.0 + mod[0:1, D:2 * D]) + mod[0:1, 0:D]).astype(bf16)

    @pl.when(i < N)
    def _():
        h = hid()
        hs[i] = h
        y = lax.dot_general(wt[D:, :], h, NT, preferred_element_type=f32)
        for g in range(2 * G):
            for t in range(T // 128):
                ph = _phi(y[64 * g:64 * g + 64, 128 * t:128 * t + 128])
                for a in range(8):
                    rows = slice(128 * g + 16 * a, 128 * g + 16 * a + 16)
                    pk[rows, 128 * t:128 * t + 128] = jnp.concatenate(
                        ph[2 * a:2 * a + 2], axis=0).astype(bf16)
            v = jnp.concatenate([y[D + 64 * g:D + 64 * g + 64].astype(bf16),
                                 jnp.ones((16, T), bf16)], axis=0)
            kv[g] += lax.dot_general(
                v, pk[128 * g:128 * g + 128, :], NT, preferred_element_type=f32)

    @pl.when(i == N)
    def _():
        cp = cps()
        for a in cp[2:]:
            a.wait()
        fold(0)
        mod[:, 2 * D:] = jnp.dot(silu_c(), wmod[:, 2 * D:], preferred_element_type=f32)
        for g in range(2 * G):
            z[128 * g:128 * g + 128, :] = jnp.broadcast_to(kv[g, 64:65, :], (128, 128)).T
            kvt[g] = jnp.where(((r & 3) == (l & 3))[:64], kv[g, :64, :], 0.0).astype(bf16)
        for g in range(G):
            wo[128 * g:128 * g + 128, :] = jnp.dot(
                perm(), wo[128 * g:128 * g + 128, :], preferred_element_type=f32).astype(bf16)

    @pl.when(i >= N)
    def _():
        y = lax.dot_general(wt[:D, :], hs[i - N], NT, preferred_element_type=f32)
        for g in range(2 * G):
            rd = []
            for t in range(T // 128):
                ph = _phi(y[64 * g:64 * g + 64, 128 * t:128 * t + 128])
                den = None
                for a in range(16):
                    w = ph[a] * z[128 * g + 8 * a:128 * g + 8 * a + 8, :]
                    den = w if den is None else den + w
                den = den + pltpu.roll(den, 4, 0)
                rd.append(jnp.tile(1.0 / (den + 1e-6), (8, 1)))
                for a in range(8):
                    pq[16 * a:16 * a + 16, 128 * t:128 * t + 128] = jnp.concatenate(
                        ph[2 * a:2 * a + 2], axis=0).astype(bf16)
            num = jnp.dot(kvt[g], pq[...], preferred_element_type=f32)
            ot[64 * g:64 * g + 64, :] = (num * jnp.concatenate(rd, axis=1)).astype(bf16)
        for q in range(T // U):
            rs = slice(q * U, q * U + U)
            att = lax.dot_general(ot[:, rs], wo[...], TN, preferred_element_type=f32)
            x1 = x_ref[rs, :].astype(f32) + mod[0:1, 2 * D:3 * D] * att
            h = (_ln(x1) * (1.0 + mod[0:1, 4 * D:5 * D]) + mod[0:1, 3 * D:4 * D]).astype(bf16)
            o_ref_x[rs, :] = x1
            hb[rs, :] = h
        for q in range(T // U2):
            rs = slice(q * U2, q * U2 + U2)
            for j in range(F // FC):
                cs = slice(j * FC, j * FC + FC)
                a = jnp.dot(hb[rs, :], wg[:, cs], preferred_element_type=f32)
                u = jnp.dot(hb[rs, :], wu[:, cs], preferred_element_type=f32)
                hf = 0.5 * a
                th = jnp.tanh(a * (0.7978845608028654 + (0.7978845608028654 * 0.044715) * (a * a)))
                act[rs, cs] = ((hf + hf * th) * u).astype(bf16)
            d = jnp.dot(act[rs, :], wd[...], preferred_element_type=f32)
            os_[i - N, rs, :] = (o_ref_x[rs, :] + mod[0:1, 5 * D:] * d).astype(os_.dtype)
            if q >= T // U2 - 2:
                ocp(i - N, q - (T // U2 - 2)).start()

        @pl.when(i == 2 * N - 1)
        def _():
            for j in range(N):
                ocp(j, 0).wait()
                ocp(j, 1).wait()


@jax.jit
def pallas_adaLN_cond__linear_kernel_hedgehog__geglu_ffn__prompt_kernel(
    A_x, A_wqkv, A_w_phi, A_wo, B_x, B_w_gate, B_w_up, B_w_down, c, w_mod,
):
    anyspec = pl.BlockSpec(memory_space=pl.ANY)
    V = pltpu.VMEM
    return pl.pallas_call(
        _kernel,
        grid=(2 * N,),
        in_specs=[
            pl.BlockSpec((None, T, D), lambda i: (0, i % N, 0)),
            pl.BlockSpec((1, D), lambda i: (0, 0)),
            pl.BlockSpec((DH, DH, H), lambda i: (0, 0, 0)),
        ] + [anyspec] * 6,
        out_specs=anyspec,
        out_shape=jax.ShapeDtypeStruct(A_x.shape, A_x.dtype),
        scratch_shapes=[
            V((D, 3 * D), bf16), V((D, 6 * D), bf16), V((D, D), bf16),
            V((D, F), bf16), V((D, F), bf16), V((F, D), bf16),
            V((3 * D, D), bf16), V((8, 6 * D), f32), V((2 * G, 80, 128), f32),
            V((2 * G, 64, 128), bf16), V((2 * D, 128), f32),
            V((2 * D, T), bf16), V((128, T), bf16), V((D, T), bf16),
            V((T, D), f32), V((T, D), bf16), V((T, F), bf16), V((G, 128, 128), bf16),
            V((N, T, D), bf16), V((N, T, D), bf16),
            pltpu.SemaphoreType.DMA((8,)), pltpu.SemaphoreType.DMA((2, N)),
        ],
        compiler_params=pltpu.CompilerParams(
            dimension_semantics=("arbitrary",), vmem_limit_bytes=100 * 1024 * 1024),
    )(A_x, c, A_w_phi.transpose(1, 2, 0), A_wqkv, w_mod, A_wo, B_w_gate, B_w_up, B_w_down)
```
